```python
import jax
import jax.numpy as jnp

def _softmax(x, axis=-1):
    return jax.nn.softmax(x, axis=axis)
def _gelu(x):
    return jax.nn.gelu(x, approximate=True)
def _silu(x):
    return jax.nn.silu(x)
def _sigmoid(x):
    return jax.nn.sigmoid(x)
def _layernorm(x, axis=-1, eps=1e-5):
    m = jnp.mean(x, axis=axis, keepdims=True)
    v = jnp.var(x, axis=axis, keepdims=True)
    return (x - m) / jnp.sqrt(v + eps)
def _scatter_add(tgt, idx, src, axis=0):
    return tgt.at[idx].add(src)
def _segment_sum(src, seg, n):
    return jax.ops.segment_sum(src, seg, n)
class _Rng:
    def __init__(self, key):
        self._k = key
    def _next(self):
        self._k, sub = jax.random.split(self._k)
        return sub
    def normal(self, shape):
        return jax.random.normal(self._next(), shape, dtype=jnp.bfloat16)
    def randint(self, lo, hi, shape):
        return jax.random.randint(self._next(), shape, lo, hi, dtype=jnp.int32)
    def uniform(self, shape, lo=0.0, hi=1.0):
        return jax.random.uniform(self._next(), shape, jnp.bfloat16, lo, hi)
    def permutation(self, n):
        return jax.random.permutation(self._next(), n)


kernel_name = 'concat_heads__compressed_kv_cla__spectral_gfnet__prompt'

def setup_inputs():
    _rng = _Rng(jax.random.key(int.from_bytes(__import__("os").urandom(4), "little")))
    _w = (lambda a: (lambda t: t.astype(jnp.bfloat16) if jnp.issubdtype(t.dtype, jnp.floating) else t)(jnp.asarray(a)))
    def _A_setup():
        B, H, Sq, Sk, D, M = 1, 32, 2048, 2048, 128, 1024
        Dc = 4 * D
        return {
            "x": _w((lambda *s: _rng.normal(s) * 0.05)(B, Sq, M)),
            "c_kv": _w((lambda *s: _rng.normal(s) * 0.05)(B, Sk, Dc)),
            "w_q": _w((lambda *s: _rng.normal(s) * 0.05)(M, H, D) * (M ** -0.5)),
            "w_uk": _w((lambda *s: _rng.normal(s) * 0.05)(Dc, H, D) * (Dc ** -0.5)),
            "w_uv": _w((lambda *s: _rng.normal(s) * 0.05)(Dc, H, D) * (Dc ** -0.5)),
            "w_o": _w((lambda *s: _rng.normal(s) * 0.05)(H, D, M) * ((H * D) ** -0.5)),
        }
    _A_in = _A_setup()

    def _B_setup():
        B, S, D = 1, 2048, 1024
        Df = D // 2 + 1
        return {
            "x": _w((lambda *s: _rng.normal(s) * 0.05)(B, S, D)),
            "w_r": _w((lambda *s: _rng.normal(s) * 0.05)(S, Df) * 0.02),
            "w_i": _w((lambda *s: _rng.normal(s) * 0.05)(S, Df) * 0.02),
        }
    _B_in = _B_setup()

    return {
        "A_x": _A_in["x"],
        "A_c_kv": _A_in["c_kv"],
        "A_w_q": _A_in["w_q"],
        "A_w_uk": _A_in["w_uk"],
        "A_w_uv": _A_in["w_uv"],
        "A_w_o": _A_in["w_o"],
        "B_x": _B_in["x"],
        "B_w_r": _B_in["w_r"],
        "B_w_i": _B_in["w_i"],
    }

def reference(A_x, A_c_kv, A_w_q, A_w_uk, A_w_uv, A_w_o, B_x, B_w_r, B_w_i):
    def _A_ref(x, c_kv, w_q, w_uk, w_uv, w_o):
        B, Sq, M = x.shape[0], x.shape[1], x.shape[2]
        Sk = c_kv.shape[1]
        H, D = w_q.shape[1], w_q.shape[2]
        q = jnp.einsum("bqm,mhd->bhqd", x, w_q)
        k = jnp.einsum("bkc,chd->bhkd", c_kv, w_uk)
        v = jnp.einsum("bkc,chd->bhkd", c_kv, w_uv)
        scores = jnp.einsum("bhqd,bhkd->bhqk", q, k) * (D ** -0.5)
        off = Sk - Sq
        qi = jnp.arange(Sq)[:, None]
        kj = jnp.arange(Sk)[None, :]
        cmask = kj <= (qi + off)
        scores = jnp.where(cmask[None, None], scores, -1e9)
        p = _softmax(scores, axis=-1)
        ctx = jnp.einsum("bhqk,bhkd->bhqd", p, v)
        return jnp.einsum("bhqd,hdm->bqm", ctx, w_o)

    def _B_ref(x, w_r, w_i):
        B, S, D = x.shape
        X = (lambda x, axes=(-2,-1): jnp.fft.rfft2(x.astype(jnp.float32), axes=axes))(x, axes=(-2, -1))
        W = w_r + 1j * w_i
        X = X * W
        y = (lambda x, s, axes=(-2,-1): jnp.fft.irfft2(x, s=s, axes=axes).astype(jnp.bfloat16))(X, (S, D), axes=(-2, -1))
        return y

    a = _A_ref(A_x, A_c_kv, A_w_q, A_w_uk, A_w_uv, A_w_o)
    b = _B_ref(B_x, B_w_r, B_w_i)
    return jnp.concatenate([a, b], axis=-1)
```

```python
import functools
import math

import jax
import jax.numpy as jnp
import ml_dtypes
import numpy as np
from jax import lax
from jax.experimental import pallas as pl
from jax.experimental.pallas import tpu as pltpu

f32 = jnp.float32
bf16 = jnp.bfloat16
u32 = jnp.uint32

S = 2048
H = 32
D = 128
M = 1024
DC = 512
QSCALE = (D ** -0.5) * math.log2(math.e)
NT = (((1,), (1,)), ((), ()))

DD = 1024
R = 32
NB = S // R
RES = ((0, 4), (1, 7), (2, 6), (3, 5))
HH = math.sqrt(0.5)


def _to_bf16(a):
    return np.ascontiguousarray(a.astype(np.float32).astype(ml_dtypes.bfloat16))


@functools.lru_cache(maxsize=None)
def _dft_consts():
    d2 = np.arange(128)

    def ang(k):
        return 2 * np.pi * ((d2[:, None] * k[None, :]) % DD) / DD

    j = np.arange(64)
    a0, a4 = ang(8 * j), ang(4 + 8 * j)
    norm = 1.0 / (S * DD)
    b0 = np.concatenate([np.cos(a0), -np.sin(a0)], axis=1)
    b0[:, 64] = (-1.0) ** d2
    b4 = np.concatenate([np.cos(a4), -np.sin(a4)], axis=1)
    g0 = np.concatenate([2 * np.cos(a0).T, -2 * np.sin(a0).T], axis=0) * norm
    g0[0, :] = norm
    g0[64, :] = (-1.0) ** d2 * norm
    g4 = np.concatenate([2 * np.cos(a4).T, -2 * np.sin(a4).T], axis=0) * norm
    fwd, inv = [], []
    for t in (1, 2, 3):
        a, b = RES[t]
        aa, ab = ang(a + 8 * j), ang(b + 8 * j)
        re = np.concatenate([np.concatenate([np.cos(aa), np.cos(ab)], 1),
                             np.concatenate([np.sin(aa), -np.sin(ab)], 1)], 0)
        im = np.concatenate([np.concatenate([-np.sin(aa), -np.sin(ab)], 1),
                             np.concatenate([np.cos(aa), -np.cos(ab)], 1)], 0)
        fwd.append(np.concatenate([re, im], axis=1))
        rows_r = np.concatenate([np.concatenate([np.cos(aa).T, np.sin(aa).T], 1),
                                 np.concatenate([np.cos(ab).T, -np.sin(ab).T], 1)], 0)
        rows_i = np.concatenate([np.concatenate([-np.sin(aa).T, np.cos(aa).T], 1),
                                 np.concatenate([-np.sin(ab).T, -np.cos(ab).T], 1)], 0)
        inv.append(np.concatenate([rows_r, rows_i], axis=0) * (2 * norm))
    fwd[0][128:, :] *= -1.0
    zeros = np.zeros((128, 128))
    dfw = np.concatenate([np.concatenate([b0, zeros], 1), np.concatenate([b4, zeros], 1)] + fwd, axis=0)
    div = np.concatenate([np.concatenate([g0, zeros], 1), np.concatenate([g4, zeros], 1)] + inv, axis=0)
    tm = np.zeros((R, 2 * NB, 2 * NB))
    k2 = np.arange(NB)[:, None]
    s2 = np.arange(NB)[None, :]
    for k1 in range(R):
        a = -2 * np.pi * ((s2 * (k1 + R * k2)) % S) / S
        tm[k1] = np.block([[np.cos(a), -np.sin(a)], [np.sin(a), np.cos(a)]])
    tmi = np.transpose(tm, (0, 2, 1))
    return (_to_bf16(dfw), _to_bf16(div),
            _to_bf16(tm.reshape(R * 2 * NB, 2 * NB)), _to_bf16(tmi.reshape(R * 2 * NB, 2 * NB)))


class _C:
    __slots__ = ("r", "i", "nr", "ni")

    def __init__(self, r, i, nr=False, ni=False):
        self.r, self.i, self.nr, self.ni = r, i, nr, ni


def _addsub(a, na, b, nb):
    if na == nb:
        return a + b, na
    if not na:
        return a - b, False
    return b - a, False


def _cadd(x, y, sub=False):
    r, nr = _addsub(x.r, x.nr, y.r, y.nr ^ sub)
    i, ni = _addsub(x.i, x.ni, y.i, y.ni ^ sub)
    return _C(r, i, nr, ni)


def _ctw(x, n, k, sign):
    k = k % n
    if k == 0:
        return x
    if 4 * k == n or 4 * k == 3 * n:
        if (4 * k == n) == (sign > 0):
            return _C(x.i, x.r, not x.ni, x.nr)
        return _C(x.i, x.r, x.ni, not x.nr)
    if 2 * k == n:
        return _C(x.r, x.i, not x.nr, not x.ni)
    a = sign * 2 * math.pi * k / n
    c, s = math.cos(a), math.sin(a)
    sr = -1.0 if x.nr else 1.0
    si = -1.0 if x.ni else 1.0
    if (8 * k) % n == 0:
        re = (x.r - x.i) if (s * si) / (c * sr) > 0 else (x.r + x.i)
        im = (x.r + x.i) if (c * si) / (s * sr) > 0 else (x.r - x.i)
        return _C(re * (c * sr), im * (s * sr))
    return _C(x.r * (c * sr) - x.i * (s * si), x.r * (s * sr) + x.i * (c * si))


def _fft_list(xs, sign):
    n = len(xs)
    if n == 1:
        return xs
    e = _fft_list(xs[0::2], sign)
    o = _fft_list(xs[1::2], sign)
    out = [None] * n
    for k in range(n // 2):
        t = _ctw(o[k], n, k, sign)
        out[k] = _cadd(e[k], t)
        out[k + n // 2] = _cadd(e[k], t, sub=True)
    return out


def _parts(x):
    return (-x.r if x.nr else x.r), (-x.i if x.ni else x.i)


def _d_fwd(xb, dfw, pr, pi, r0, rows):
    sl = pl.ds(r0, rows)
    x = [xb[sl, d * 128:(d + 1) * 128].astype(f32) for d in range(8)]
    a0 = x[0] + x[4]; a1 = x[0] - x[4]; b0 = x[2] + x[6]; b1 = x[2] - x[6]
    c0 = x[1] + x[5]; c1 = x[1] - x[5]; d0 = x[3] + x[7]; d1 = x[3] - x[7]
    e0 = a0 + b0; f0 = c0 + d0
    A0 = e0 + f0; A4 = e0 - f0
    A2r = a0 - b0; A2i = d0 - c0
    g = (c1 - d1) * HH; hh = (c1 + d1) * HH
    A1r = a1 + g; A1n = b1 + hh
    A3r = a1 - g; A3i = b1 - hh
    p0 = jnp.dot(A0.astype(bf16), dfw[0:128, 0:128], preferred_element_type=f32)
    p4 = jnp.dot(A4.astype(bf16), dfw[128:256, 0:128], preferred_element_type=f32)
    lane = lax.broadcasted_iota(jnp.int32, (rows, 128), 1)
    lo = lane < 64
    t0r = jnp.where(lo, p0, pltpu.roll(p4, 64, 1))
    t0i = jnp.where(lo, pltpu.roll(p0, 64, 1), p4)
    pr[0, sl, :] = t0r
    pi[0, sl, :] = jnp.where(lane == 0, 0.0, t0i)
    pr[4, sl, :] = jnp.where(lane == 0, t0i, 0.0)
    pi[4, sl, :] = jnp.zeros((rows, 128), f32)
    for t, (ar, ai) in enumerate(((A1r, A1n), (A2r, A2i), (A3r, A3i)), start=1):
        lhs = jnp.concatenate([ar, ai], axis=1).astype(bf16)
        o = jnp.dot(lhs, dfw[t * 256:(t + 1) * 256, :], preferred_element_type=f32)
        pr[t, sl, :] = o[:, 0:128]
        pi[t, sl, :] = o[:, 128:256]


def _d_inv(pr, pi, div, out, r0, rows):
    sl = pl.ds(r0, rows)
    lane = lax.broadcasted_iota(jnp.int32, (rows, 128), 1)
    lo = lane < 64
    v0r = pr[0, sl, :]
    v0i = jnp.where(lane == 0, pr[4, sl, :], pi[0, sl, :])
    l0 = jnp.where(lo, v0r, pltpu.roll(v0i, 64, 1))
    l4 = jnp.where(lo, pltpu.roll(v0r, 64, 1), v0i)
    C0 = jnp.dot(l0.astype(bf16), div[0:128, 0:128], preferred_element_type=f32)
    C4 = jnp.dot(l4.astype(bf16), div[128:256, 0:128], preferred_element_type=f32)
    cc = []
    for t in (1, 2, 3):
        lhs = jnp.concatenate([pr[t, sl, :], pi[t, sl, :]], axis=1).astype(bf16)
        o = jnp.dot(lhs, div[t * 256:(t + 1) * 256, :], preferred_element_type=f32)
        cc.append((o[:, 0:128], o[:, 128:256]))
    (C1r, C1i), (C2r, C2i), (C3r, C3i) = cc
    s04 = C0 + C4; d04 = C0 - C4
    E = [s04 + C2r, d04 - C2i, s04 - C2r, d04 + C2i]
    u = C1r - C3r; v = C1i + C3i
    O0 = C1r + C3r; O2 = C3i - C1i; O1 = (u - v) * HH; O3n = (u + v) * HH
    ys = [E[0] + O0, E[1] + O1, E[2] + O2, E[3] - O3n, E[0] - O0, E[1] - O1, E[2] - O2, E[3] + O3n]
    for d in range(8):
        out[sl, d * 128:(d + 1) * 128] = ys[d].astype(bf16)


def _w_prep(wt3, wny, wb, t, jt):
    c0 = jt * 128
    if t < 4:
        w32 = wt3.at[jt].bitcast(u32)
        parts = []
        for res in RES[t]:
            w = w32[pl.ds(res // 2, 64, stride=4), :]
            w = (w << 16) if res % 2 == 0 else (w & jnp.uint32(0xFFFF0000))
            parts.append(pltpu.bitcast(w, f32))
        tile = jnp.concatenate(parts, axis=0).astype(bf16)
    else:
        tile = jnp.broadcast_to(wny[0:1, c0:c0 + 128], (128, 128))
    wb[t, c0:c0 + 128, :] = tile.T


def _stage_a(pr, pi, t, g, sign):
    xs = [_C(pr[t, pl.ds(s1 * NB + g * 8, 8), :], pi[t, pl.ds(s1 * NB + g * 8, 8), :]) for s1 in range(R)]
    ys = _fft_list(xs, sign)
    for k1 in range(R):
        r, i = _parts(ys[k1])
        pr[t, pl.ds(k1 * NB + g * 8, 8), :] = r
        pi[t, pl.ds(k1 * NB + g * 8, 8), :] = i


def _stage_b(pr, pi, tm, tmi, wbr, wbi, t, p0):
    wr = wbr.at[t].bitcast(u32)[pl.ds(p0, NB, stride=R // 2), :]
    wi = wbi.at[t].bitcast(u32)[pl.ds(p0, NB, stride=R // 2), :]
    for half in range(2):
        k1 = 2 * p0 + half
        if half == 0:
            fr = pltpu.bitcast(wr << 16, f32)
            fi = pltpu.bitcast(wi << 16, f32)
        else:
            fr = pltpu.bitcast(wr & jnp.uint32(0xFFFF0000), f32)
            fi = pltpu.bitcast(wi & jnp.uint32(0xFFFF0000), f32)
        blk = pl.ds(k1 * NB, NB)
        a = jnp.concatenate([pr[t, blk, :], pi[t, blk, :]], axis=0).astype(bf16)
        x = jnp.dot(tm[k1 * 128:(k1 + 1) * 128, :], a, preferred_element_type=f32)
        xr, xi = x[:NB], x[NB:]
        u = jnp.concatenate([xr * fr - xi * fi, xr * fi + xi * fr], axis=0).astype(bf16)
        c = jnp.dot(tmi[k1 * 128:(k1 + 1) * 128, :], u, preferred_element_type=f32)
        pr[t, blk, :] = c[:NB]
        pi[t, blk, :] = c[NB:]


def _s_pieces(pr, pi, tm, tmi, wbr, wbi, t):
    ps = [functools.partial(_stage_a, pr, pi, t, g, -1) for g in range(NB // 8)]
    ps += [functools.partial(_stage_b, pr, pi, tm, tmi, wbr, wbi, t, p0) for p0 in range(R // 2)]
    ps += [functools.partial(_stage_a, pr, pi, t, g, +1) for g in range(NB // 8)]
    return ps


class _Filler:
    def __init__(self, pieces):
        self.p = list(pieces)
        self.done = 0

    def upto(self, frac):
        tgt = int(round(frac * len(self.p)))
        while self.done < tgt:
            self.p[self.done]()
            self.done += 1


def _head_weights(words, parity):
    w = (words << 16) if parity == 0 else (words & jnp.uint32(0xFFFF0000))
    return pltpu.bitcast(w, f32).astype(bf16)


def _proj_pieces(xa, cb, wq, wk, wv, slot, parity, q_dst, kv_dst, rows=256):
    st = {}
    n = S // rows

    def mk_kv(r):
        def f():
            if r == 0:
                st["kv"] = jnp.concatenate([_head_weights(wk[slot], parity), _head_weights(wv[slot], parity)], axis=1)
            kv = jnp.dot(cb[r * rows:(r + 1) * rows, :], st["kv"], preferred_element_type=f32)
            kv_dst[r * rows:(r + 1) * rows, :] = kv.astype(bf16)
        return f

    def mk_q(r):
        def f():
            if r == 0:
                st["q"] = _head_weights(wq[slot], parity)
            q = jnp.dot(xa[r * rows:(r + 1) * rows, :], st["q"], preferred_element_type=f32)
            q_dst[r * rows:(r + 1) * rows, :] = (q * QSCALE).astype(bf16)
        return f

    return [mk_kv(r) for r in range(n)] + [mk_q(r) for r in range(n)]


def _fold(s, op):
    r = s[:, 0:128]
    for c in range(1, s.shape[1] // 128):
        r = op(r, s[:, c * 128:(c + 1) * 128])
    return r


def _recip(l):
    r = pl.reciprocal(l, approx=True)
    return r * (2.0 - l * r)


def _attention(q_ref, kv_ref, ctx, col0, pieces, bq=128, bk=512):
    nq = S // bq
    fill = _Filler(pieces)
    ntiles = lambda i: ((i + 1) * bq + bk - 1) // bk
    width = lambda i, t: min(bk, (i + 1) * bq - t * bk)

    def qk_tile(i, t, q):
        w = width(i, t)
        s = lax.dot_general(q, kv_ref[t * bk:t * bk + w, 0:D], NT, preferred_element_type=f32)
        if t * bk + w - 1 > i * bq:
            row = lax.broadcasted_iota(jnp.int32, (bq, bq), 0)
            col = lax.broadcasted_iota(jnp.int32, (bq, bq), 1)
            diag = jnp.where(col <= row, s[:, w - bq:], -1e9)
            s = diag if w == bq else jnp.concatenate([s[:, :w - bq], diag], axis=1)
        return s

    def do_round(i, s_cur, m_cur):
        s_nxt, mvec, lvec, acc = [], None, None, None
        n_cur = ntiles(i) if i >= 0 else 0
        n_nxt = ntiles(i + 1) if i + 1 < nq else 0
        if n_nxt:
            qn = q_ref[(i + 1) * bq:(i + 2) * bq, :]
        for t in range(max(n_cur, n_nxt)):
            if t < n_nxt:
                s = qk_tile(i + 1, t, qn)
                s_nxt.append(s)
                f = _fold(s, jnp.maximum)
                mvec = f if mvec is None else jnp.maximum(mvec, f)
            if t < n_cur:
                w = width(i, t)
                p = jnp.exp2(s_cur[t] - m_cur)
                f = _fold(p, jnp.add)
                lvec = f if lvec is None else lvec + f
                o = jnp.dot(p.astype(bf16), kv_ref[t * bk:t * bk + w, D:2 * D], preferred_element_type=f32)
                acc = o if acc is None else acc + o
        m_nxt = jnp.max(mvec, axis=1, keepdims=True) if n_nxt else None
        if i >= 0:
            l = jnp.sum(lvec, axis=1, keepdims=True)
            ctx[i * bq:(i + 1) * bq, pl.ds(col0, D)] = (acc * _recip(l)).astype(bf16)
        fill.upto((i + 2) / (nq + 1))
        return s_nxt, m_nxt

    s_cur, m_cur = do_round(-1, None, None)
    for i in range(nq):
        s_cur, m_cur = do_round(i, s_cur, m_cur)
    fill.upto(1.0)


OROW = 512


def _kernel(x_h, c_h, wq_h, wk_h, wv_h, wo_h, xb_h, wr_h, wi_h, dfw_h, div_h, tm_h, tmi_h, out_h,
            xa, cb, wq, wk, wv, wo, qa, kva, qb, kvb, ctx,
            xb, wtr, wti, wnr, wni, dfw, div, tm, tmi, pr, pi, wbr, wbi,
            sem_a, sem_w, sem_b, sem_o):
    def wcopies(pair, slot):
        return (pltpu.make_async_copy(wk_h.bitcast(u32).at[:, pair, :], wk.at[slot], sem_w.at[slot, 0]),
                pltpu.make_async_copy(wv_h.bitcast(u32).at[:, pair, :], wv.at[slot], sem_w.at[slot, 1]),
                pltpu.make_async_copy(wq_h.bitcast(u32).at[:, pair, :], wq.at[slot], sem_w.at[slot, 2]))

    c_cp = pltpu.make_async_copy(c_h, cb, sem_a.at[0])
    x_cp = pltpu.make_async_copy(x_h, xa, sem_a.at[1])
    wo_cp = pltpu.make_async_copy(wo_h, wo, sem_a.at[2])
    b_cps = [pltpu.make_async_copy(a, b, sem_b.at[i]) for i, (a, b) in enumerate(
        ((xb_h, xb), (dfw_h, dfw), (div_h, div), (tm_h, tm), (tmi_h, tmi),
         (wr_h.at[512:513, :], wnr), (wi_h.at[512:513, :], wni)))]

    w0 = wcopies(0, 0)
    c_cp.start(); w0[0].start(); w0[1].start()
    x_cp.start(); w0[2].start()
    for cp in wcopies(1, 1):
        cp.start()
    for cp in b_cps:
        cp.start()
    for jt in range(16):
        pltpu.make_async_copy(wr_h.at[0:512, jt * 128:(jt + 1) * 128], wtr.at[jt], sem_b.at[7]).start()
        pltpu.make_async_copy(wi_h.at[0:512, jt * 128:(jt + 1) * 128], wti.at[jt], sem_b.at[8]).start()
    wo_cp.start()

    proj = functools.partial(_proj_pieces, xa, cb, wq, wk, wv)
    first = proj(0, 0, qa, kva)
    c_cp.wait(); w0[0].wait(); w0[1].wait()
    for f in first[:8]:
        f()
    x_cp.wait(); w0[2].wait()
    for f in first[8:]:
        f()

    def pair_body(p, last):
        if not last:
            for cp in wcopies(p + 1, lax.rem(p + 1, 3)):
                cp.wait()

            @pl.when(p + 2 < H // 2)
            def _():
                for cp in wcopies(p + 2, lax.rem(p + 2, 3)):
                    cp.start()
        else:
            for cp in b_cps:
                cp.wait()
            pltpu.make_async_copy(wtr, wtr, sem_b.at[7]).wait()
            pltpu.make_async_copy(wti, wti, sem_b.at[8]).wait()
        col = pl.multiple_of(p * 2 * D, 2 * D)
        fa = proj(lax.rem(p, 3), 1, qb, kvb)
        if last:
            fa = fa + [functools.partial(_w_prep, wt, wn, wb, t, jt)
                       for t in range(5) for jt in range(16) for (wt, wn, wb) in ((wtr, wnr, wbr), (wti, wni, wbi))]
        _attention(qa, kva, ctx, col, fa)
        if last:
            fb = [functools.partial(_d_fwd, xb, dfw, pr, pi, r * 128, 128) for r in range(S // 128)]
            fb += _s_pieces(pr, pi, tm, tmi, wbr, wbi, 4)
        else:
            fb = proj(lax.rem(p + 1, 3), 0, qa, kva)
        _attention(qb, kvb, ctx, pl.multiple_of(p * 2 * D + D, D), fb)

    def loop_body(p, carry):
        pair_body(p, False)
        return carry

    lax.fori_loop(0, H // 2 - 1, loop_body, 0)
    pair_body(H // 2 - 1, True)
    wo_cp.wait()

    def out_body(r, carry):
        row0 = pl.multiple_of(r * OROW, OROW)
        pieces = _s_pieces(pr, pi, tm, tmi, wbr, wbi, r)
        fill = _Filler(pieces)
        sub = 128
        for j in range(OROW // sub):
            rows = pl.ds(row0 + j * sub, sub)
            o = jnp.dot(ctx[rows, :], wo[...], preferred_element_type=f32)
            xa[rows, :] = o.astype(bf16)
            fill.upto((j + 1) / (OROW // sub))
        pltpu.make_async_copy(xa.at[pl.ds(row0, OROW), :], out_h.at[pl.ds(row0, OROW), 0:M], sem_o.at[r]).start()
        return carry

    lax.fori_loop(0, S // OROW, out_body, 0)

    nchunk = 4
    ycp = []
    for r in range(nchunk):
        for j in range(S // nchunk // 128):
            _d_inv(pr, pi, div, xb, r * (S // nchunk) + j * 128, 128)
        rows = slice(r * (S // nchunk), (r + 1) * (S // nchunk))
        cp = pltpu.make_async_copy(xb.at[rows, :], out_h.at[rows, M:M + DD], sem_o.at[4 + r])
        cp.start()
        ycp.append(cp)
    for r in range(S // OROW):
        pltpu.make_async_copy(xa.at[pl.ds(r * OROW, OROW), :], out_h.at[pl.ds(r * OROW, OROW), 0:M], sem_o.at[r]).wait()
    for cp in ycp:
        cp.wait()


@jax.jit
def pallas_concat_heads__compressed_kv_cla__spectral_gfnet__prompt_kernel(
        A_x, A_c_kv, A_w_q, A_w_uk, A_w_uv, A_w_o, B_x, B_w_r, B_w_i):
    dfw, div, tm, tmi = _dft_consts()
    hbm = pl.BlockSpec(memory_space=pl.ANY)
    vm = pltpu.VMEM
    scratch = [
        vm((S, M), bf16), vm((S, DC), bf16),
        vm((3, M, D), u32), vm((3, DC, D), u32), vm((3, DC, D), u32), vm((H * D, M), bf16),
        vm((S, D), bf16), vm((S, 2 * D), bf16), vm((S, D), bf16), vm((S, 2 * D), bf16), vm((S, H * D), bf16),
        vm((S, DD), bf16), vm((16, 512, 128), bf16), vm((16, 512, 128), bf16), vm((1, S), bf16), vm((1, S), bf16),
        vm((1024, 256), bf16), vm((1024, 256), bf16), vm((R * 128, 128), bf16), vm((R * 128, 128), bf16),
        vm((5, S, 128), f32), vm((5, S, 128), f32), vm((5, S, 128), bf16), vm((5, S, 128), bf16),
        pltpu.SemaphoreType.DMA((3,)), pltpu.SemaphoreType.DMA((3, 3)),
        pltpu.SemaphoreType.DMA((9,)), pltpu.SemaphoreType.DMA((8,)),
    ]
    out = pl.pallas_call(
        _kernel,
        out_shape=jax.ShapeDtypeStruct((S, M + DD), bf16),
        in_specs=[hbm] * 13,
        out_specs=hbm,
        scratch_shapes=scratch,
        compiler_params=pltpu.CompilerParams(vmem_limit_bytes=124 * 1024 * 1024),
        name="mla_gfnet",
    )(A_x.reshape(S, M), A_c_kv.reshape(S, DC), A_w_q, A_w_uk, A_w_uv, A_w_o.reshape(H * D, M),
      B_x.reshape(S, DD), B_w_r.T, B_w_i.T,
      jnp.asarray(dfw), jnp.asarray(div), jnp.asarray(tm), jnp.asarray(tmi))
    return out.reshape(1, S, M + DD)
```

```python
import contextlib
import functools
import math

import jax
import jax.numpy as jnp
import ml_dtypes
import numpy as np
from jax import lax
from jax.experimental import pallas as pl
from jax.experimental.pallas import tpu as pltpu

f32 = jnp.float32
bf16 = jnp.bfloat16
u32 = jnp.uint32

CFG = {"ychunk": 2}


def _scope(name):
    inner = name.startswith(("pa", "pb", "top"))
    on = CFG.get("scopes", 0) >= (2 if inner else 1)
    return jax.named_scope(name) if on else contextlib.nullcontext()


S = 2048
H = 32
D = 128
M = 1024
DC = 512
QSCALE = (D ** -0.5) * math.log2(math.e)
NT = (((1,), (1,)), ((), ()))
SAFE_LOG2 = CFG.get("safe", 64.0)

DD = 1024
R = 32
NB = S // R
RES = ((0, 4), (1, 7), (2, 6), (3, 5))
HH = math.sqrt(0.5)


def _to_bf16(a):
    return np.ascontiguousarray(a.astype(np.float32).astype(ml_dtypes.bfloat16))


@functools.lru_cache(maxsize=None)
def _dft_consts():
    d2 = np.arange(128)

    def ang(k):
        return 2 * np.pi * ((d2[:, None] * k[None, :]) % DD) / DD

    j = np.arange(64)
    a0, a4 = ang(8 * j), ang(4 + 8 * j)
    norm = 1.0 / (S * DD)
    b0 = np.concatenate([np.cos(a0), -np.sin(a0)], axis=1)
    b0[:, 64] = (-1.0) ** d2
    b4 = np.concatenate([np.cos(a4), -np.sin(a4)], axis=1)
    g0 = np.concatenate([2 * np.cos(a0).T, -2 * np.sin(a0).T], axis=0) * norm
    g0[0, :] = norm
    g0[64, :] = (-1.0) ** d2 * norm
    g4 = np.concatenate([2 * np.cos(a4).T, -2 * np.sin(a4).T], axis=0) * norm
    fwd, inv = [], []
    for t in (1, 2, 3):
        a, b = RES[t]
        aa, ab = ang(a + 8 * j), ang(b + 8 * j)
        re = np.concatenate([np.concatenate([np.cos(aa), np.cos(ab)], 1),
                             np.concatenate([np.sin(aa), -np.sin(ab)], 1)], 0)
        im = np.concatenate([np.concatenate([-np.sin(aa), -np.sin(ab)], 1),
                             np.concatenate([np.cos(aa), -np.cos(ab)], 1)], 0)
        fwd.append(np.concatenate([re, im], axis=1))
        rows_r = np.concatenate([np.concatenate([np.cos(aa).T, np.sin(aa).T], 1),
                                 np.concatenate([np.cos(ab).T, -np.sin(ab).T], 1)], 0)
        rows_i = np.concatenate([np.concatenate([-np.sin(aa).T, np.cos(aa).T], 1),
                                 np.concatenate([-np.sin(ab).T, -np.cos(ab).T], 1)], 0)
        inv.append(np.concatenate([rows_r, rows_i], axis=0) * (2 * norm))
    fwd[0][128:, :] *= -1.0
    zeros = np.zeros((128, 128))
    dfw = np.concatenate([np.concatenate([b0, zeros], 1), np.concatenate([b4, zeros], 1)] + fwd, axis=0)
    div = np.concatenate([np.concatenate([g0, zeros], 1), np.concatenate([g4, zeros], 1)] + inv, axis=0)
    tm = np.zeros((R, 2 * NB, 2 * NB))
    k2 = np.arange(NB)[:, None]
    s2 = np.arange(NB)[None, :]
    for k1 in range(R):
        a = -2 * np.pi * ((s2 * (k1 + R * k2)) % S) / S
        tm[k1] = np.block([[np.cos(a), -np.sin(a)], [np.sin(a), np.cos(a)]])
    tmi = np.transpose(tm, (0, 2, 1))
    return (_to_bf16(dfw), _to_bf16(div),
            _to_bf16(tm.reshape(R * 2 * NB, 2 * NB)), _to_bf16(tmi.reshape(R * 2 * NB, 2 * NB)))


def _mo(v, n):
    return v if isinstance(v, int) else pl.multiple_of(v, n)


def _half(r0):
    return r0 // 2 if isinstance(r0, int) else pl.multiple_of(r0 >> 1, 8)


def _ld(ref, r0, n, cols=slice(None)):
    return pltpu.bitcast(ref[pl.ds(_half(r0), n // 2), cols], bf16)


def _st(ref, r0, n, cols, val):
    ref[pl.ds(_half(r0), n // 2), cols] = pltpu.bitcast(val.astype(bf16), u32)


class _C:
    __slots__ = ("r", "i", "nr", "ni")

    def __init__(self, r, i, nr=False, ni=False):
        self.r, self.i, self.nr, self.ni = r, i, nr, ni


def _addsub(a, na, b, nb):
    if na == nb:
        return a + b, na
    if not na:
        return a - b, False
    return b - a, False


def _cadd(x, y, sub=False):
    r, nr = _addsub(x.r, x.nr, y.r, y.nr ^ sub)
    i, ni = _addsub(x.i, x.ni, y.i, y.ni ^ sub)
    return _C(r, i, nr, ni)


def _ctw(x, n, k, sign):
    k = k % n
    if k == 0:
        return x
    if 4 * k == n or 4 * k == 3 * n:
        if (4 * k == n) == (sign > 0):
            return _C(x.i, x.r, not x.ni, x.nr)
        return _C(x.i, x.r, x.ni, not x.nr)
    if 2 * k == n:
        return _C(x.r, x.i, not x.nr, not x.ni)
    a = sign * 2 * math.pi * k / n
    c, s = math.cos(a), math.sin(a)
    sr = -1.0 if x.nr else 1.0
    si = -1.0 if x.ni else 1.0
    if (8 * k) % n == 0:
        re = (x.r - x.i) if (s * si) / (c * sr) > 0 else (x.r + x.i)
        im = (x.r + x.i) if (c * si) / (s * sr) > 0 else (x.r - x.i)
        return _C(re * (c * sr), im * (s * sr))
    return _C(x.r * (c * sr) - x.i * (s * si), x.r * (s * sr) + x.i * (c * si))


def _fft_list(xs, sign):
    n = len(xs)
    if n == 1:
        return xs
    e = _fft_list(xs[0::2], sign)
    o = _fft_list(xs[1::2], sign)
    out = [None] * n
    for k in range(n // 2):
        t = _ctw(o[k], n, k, sign)
        out[k] = _cadd(e[k], t)
        out[k + n // 2] = _cadd(e[k], t, sub=True)
    return out


def _parts(x):
    return (-x.r if x.nr else x.r), (-x.i if x.ni else x.i)


class _PView:
    def __init__(self, big, base):
        self.big, self.base = big, base

    def _loc(self, idx):
        t, sl = idx[0], idx[1]
        r0, n = sl.start, sl.size
        if isinstance(r0, int):
            return self.base + 2 * t + r0 // 1024, pl.ds(r0 % 1024, n)
        return self.base + 2 * t + (r0 >> 10), pl.ds(pl.multiple_of(r0 & 1023, 8), n)

    def __getitem__(self, idx):
        plane, rows = self._loc(idx)
        return pltpu.bitcast(self.big[plane, rows, :], f32)

    def __setitem__(self, idx, val):
        plane, rows = self._loc(idx)
        self.big[plane, rows, :] = pltpu.bitcast(val, u32)


def _d_fwd(xb, dfw, pr, pi, r0, rows):
    sl = pl.ds(r0, rows)
    x = [_ld(xb, r0, rows, slice(d * 128, (d + 1) * 128)).astype(f32) for d in range(8)]
    a0 = x[0] + x[4]; a1 = x[0] - x[4]; b0 = x[2] + x[6]; b1 = x[2] - x[6]
    c0 = x[1] + x[5]; c1 = x[1] - x[5]; d0 = x[3] + x[7]; d1 = x[3] - x[7]
    e0 = a0 + b0; f0 = c0 + d0
    A0 = e0 + f0; A4 = e0 - f0
    A2r = a0 - b0; A2i = d0 - c0
    g = (c1 - d1) * HH; hh = (c1 + d1) * HH
    A1r = a1 + g; A1n = b1 + hh
    A3r = a1 - g; A3i = b1 - hh
    p0 = jnp.dot(A0.astype(bf16), _ld(dfw, 0, 128, slice(0, 128)), preferred_element_type=f32)
    p4 = jnp.dot(A4.astype(bf16), _ld(dfw, 128, 128, slice(0, 128)), preferred_element_type=f32)
    lane = lax.broadcasted_iota(jnp.int32, (rows, 128), 1)
    lo = lane < 64
    t0r = jnp.where(lo, p0, pltpu.roll(p4, 64, 1))
    t0i = jnp.where(lo, pltpu.roll(p0, 64, 1), p4)
    pr[0, sl, :] = t0r
    pi[0, sl, :] = jnp.where(lane == 0, 0.0, t0i)
    pr[4, sl, :] = jnp.where(lane == 0, t0i, 0.0)
    pi[4, sl, :] = jnp.zeros((rows, 128), f32)
    for t, (ar, ai) in enumerate(((A1r, A1n), (A2r, A2i), (A3r, A3i)), start=1):
        lhs = jnp.concatenate([ar, ai], axis=1).astype(bf16)
        o = jnp.dot(lhs, _ld(dfw, t * 256, 256), preferred_element_type=f32)
        pr[t, sl, :] = o[:, 0:128]
        pi[t, sl, :] = o[:, 128:256]


def _d_inv(pr, pi, div, out, r0, rows):
    sl = pl.ds(r0, rows)
    lane = lax.broadcasted_iota(jnp.int32, (rows, 128), 1)
    lo = lane < 64
    v0r = pr[0, sl, :]
    v0i = jnp.where(lane == 0, pr[4, sl, :], pi[0, sl, :])
    l0 = jnp.where(lo, v0r, pltpu.roll(v0i, 64, 1))
    l4 = jnp.where(lo, pltpu.roll(v0r, 64, 1), v0i)
    C0 = jnp.dot(l0.astype(bf16), _ld(div, 0, 128, slice(0, 128)), preferred_element_type=f32)
    C4 = jnp.dot(l4.astype(bf16), _ld(div, 128, 128, slice(0, 128)), preferred_element_type=f32)
    cc = []
    for t in (1, 2, 3):
        lhs = jnp.concatenate([pr[t, sl, :], pi[t, sl, :]], axis=1).astype(bf16)
        o = jnp.dot(lhs, _ld(div, t * 256, 256), preferred_element_type=f32)
        cc.append((o[:, 0:128], o[:, 128:256]))
    (C1r, C1i), (C2r, C2i), (C3r, C3i) = cc
    s04 = C0 + C4; d04 = C0 - C4
    E = [s04 + C2r, d04 - C2i, s04 - C2r, d04 + C2i]
    u = C1r - C3r; v = C1i + C3i
    O0 = C1r + C3r; O2 = C3i - C1i; O1 = (u - v) * HH; O3n = (u + v) * HH
    ys = [E[0] + O0, E[1] + O1, E[2] + O2, E[3] - O3n, E[0] - O0, E[1] - O1, E[2] - O2, E[3] + O3n]
    for d in range(8):
        _st(out, r0, rows, slice(d * 128, (d + 1) * 128), ys[d])


def _w_prep(wt3, wny, wb, t, jt):
    c0 = _mo(jt * 128, 128)
    if t < 4:
        w32 = wt3.at[jt].bitcast(u32)
        parts = []
        for res in RES[t]:
            w = w32[pl.ds(res // 2, 64, stride=4), :]
            w = (w << 16) if res % 2 == 0 else (w & jnp.uint32(0xFFFF0000))
            parts.append(pltpu.bitcast(w, f32))
        tile = jnp.concatenate(parts, axis=0).astype(bf16)
    else:
        tile = jnp.broadcast_to(wny[0:1, pl.ds(c0, 128)], (128, 128))
    wb[t, pl.ds(c0, 128), :] = tile.T


def _blk(k1):
    return 8 * (k1 % 4) + k1 // 4


def _rd(pr, pi, t, blk, g):
    sl = pl.ds(blk * NB + g * 8, 8)
    return _C(pr[t, sl, :], pi[t, sl, :])


def _wr(pr, pi, t, blk, g, val):
    sl = pl.ds(blk * NB + g * 8, 8)
    r, i = _parts(val)
    pr[t, sl, :] = r
    pi[t, sl, :] = i


def _radix4(pr, pi, t, g, b, sign):
    xs = [_rd(pr, pi, t, 8 * a + b, g) for a in range(4)]
    if sign > 0:
        xs = [_ctw(xs[c], 32, b * c, sign) for c in range(4)]
    ys = _fft_list(xs, sign)
    if sign < 0:
        ys = [_ctw(ys[c], 32, b * c, sign) for c in range(4)]
    for c in range(4):
        _wr(pr, pi, t, 8 * c + b, g, ys[c])


def _radix8(pr, pi, t, g, c, sign):
    xs = [_rd(pr, pi, t, 8 * c + b, g) for b in range(8)]
    ys = _fft_list(xs, sign)
    for e in range(8):
        _wr(pr, pi, t, 8 * c + e, g, ys[e])


def _stage_b1(pr, pi, tm, wbr, wbi, t, p0):
    wr = wbr.at[t].bitcast(u32)[pl.ds(p0, NB, stride=R // 2), :]
    wi = wbi.at[t].bitcast(u32)[pl.ds(p0, NB, stride=R // 2), :]
    for half in range(2):
        k1 = 2 * p0 + half
        if half == 0:
            fr = pltpu.bitcast(wr << 16, f32)
            fi = pltpu.bitcast(wi << 16, f32)
        else:
            fr = pltpu.bitcast(wr & jnp.uint32(0xFFFF0000), f32)
            fi = pltpu.bitcast(wi & jnp.uint32(0xFFFF0000), f32)
        blk = pl.ds(_blk(k1) * NB, NB)
        a = jnp.concatenate([pr[t, blk, :], pi[t, blk, :]], axis=0).astype(bf16)
        x = jnp.dot(_ld(tm, k1 * 128, 128), a, preferred_element_type=f32)
        xr, xi = x[:NB], x[NB:]
        pr[t, blk, :] = xr * fr - xi * fi
        pi[t, blk, :] = xr * fi + xi * fr


def _stage_b2(pr, pi, tmi, t, p0):
    for k1 in (2 * p0, 2 * p0 + 1):
        blk = pl.ds(_blk(k1) * NB, NB)
        u = jnp.concatenate([pr[t, blk, :], pi[t, blk, :]], axis=0).astype(bf16)
        c = jnp.dot(_ld(tmi, k1 * 128, 128), u, preferred_element_type=f32)
        pr[t, blk, :] = c[:NB]
        pi[t, blk, :] = c[NB:]


def _s_fwd(pr, pi, ts):
    P = functools.partial
    NG = NB // 8
    ps = []
    for g in range(NG):
        ps += [(1, P(_radix4, pr, pi, ts[0], g, b, -1)) for b in range(8)]
    for g in range(NG):
        ps += [(2, P(_radix8, pr, pi, ts[1], g, c, -1)) for c in range(4)]
    return ps


def _s_rest(pr, pi, tm, tmi, wbr, wbi, ts):
    P = functools.partial
    NG = NB // 8
    ps = []
    ps += [(CFG.get("cb1", 5), P(_stage_b1, pr, pi, tm, wbr, wbi, ts[2], p0)) for p0 in range(R // 2)]
    ps += [(CFG.get("cb2", 3), P(_stage_b2, pr, pi, tmi, ts[3], p0)) for p0 in range(R // 2)]
    for g in range(NG):
        ps += [(2, P(_radix8, pr, pi, ts[4], g, c, +1)) for c in range(4)]
    for g in range(NG):
        ps += [(1, P(_radix4, pr, pi, ts[5], g, b, +1)) for b in range(8)]
    return ps


class _Filler:
    def __init__(self, pieces):
        self.p = list(pieces)
        self.total = float(sum(c for c, _ in self.p))
        self.done = 0
        self.spent = 0.0

    def insert(self, pieces):
        self.p[self.done:self.done] = list(pieces)
        self.total += float(sum(c for c, _ in pieces))

    def upto(self, frac):
        while self.done < len(self.p) and (frac >= 1.0 or self.spent + 0.5 * self.p[self.done][0] <= frac * self.total):
            self.spent += self.p[self.done][0]
            self.p[self.done][1]()
            self.done += 1


A_COMB = (((0, 1), (3, 1)), ((2, 1), (3, 1)), ((0, 1),), ((3, 1),), ((0, 1), (1, 1)), ((2, 1), (0, -1)), ((1, 1), (3, -1)))
B_COMB = (((0, 1), (3, 1)), ((0, 1),), ((1, 1), (3, -1)), ((2, 1), (0, -1)), ((3, 1),), ((0, 1), (1, 1)), ((2, 1), (3, 1)))
C_COMB = (((0, 1), (3, 1), (4, -1), (6, 1)), ((2, 1), (4, 1)), ((1, 1), (3, 1)), ((0, 1), (1, -1), (2, 1), (5, 1)))
A_SUMS = (0, 1, 4, 5, 6)
B_SUMS = (0, 2, 3, 5, 6)
PROD_ORDER = (2, 3, 0, 1, 4, 5, 6)


def _comb(blocks, terms):
    out = blocks[terms[0][0]]
    for idx, sg in terms[1:]:
        out = out + blocks[idx] if sg > 0 else out - blocks[idx]
    return out


def _strassen_steps(prod, finish, cost):
    c = [None] * 4

    def mk(i):
        def f():
            m = prod(i)
            for j, terms in enumerate(C_COMB):
                for idx, sg in terms:
                    if idx == i:
                        if c[j] is None:
                            c[j] = (m, sg)
                        elif c[j][1] == sg:
                            c[j] = (c[j][0] + m, sg)
                        else:
                            c[j] = (c[j][0] - m, c[j][1])
            if i == PROD_ORDER[-1]:
                finish([v if sg > 0 else -v for v, sg in c])
        return f

    return [(cost, mk(i)) for i in PROD_ORDER]


def _half_words(words, parity):
    w = (words << 16) if parity == 0 else (words & jnp.uint32(0xFFFF0000))
    return pltpu.bitcast(w, f32)


def _head_weights(words, parity):
    return _half_words(words, parity).astype(bf16)


def _left_sums(src, dst, kh, r0, n):
    g = CFG.get("sgran", 32)
    for r in range(r0, r0 + n, g):
        for c in range(0, kh, 128):
            blk = [_ld(src, r + (S // 2) * (b // 2), g, slice((b % 2) * kh + c, (b % 2) * kh + c + 128)).astype(f32)
                   for b in range(4)]
            for s_, i in enumerate(A_SUMS):
                _st(dst.at[s_], r, g, slice(c, c + 128), _comb(blk, A_COMB[i]))


def _left_operand(src, sums, kh, i, r0, n):
    if i in A_SUMS:
        return _ld(sums.at[A_SUMS.index(i)], r0, n)
    b = A_COMB[i][0][0]
    return _ld(src, r0 + (S // 2) * (b // 2), n, slice((b % 2) * kh, (b % 2 + 1) * kh))


class _RowNorm:
    def __init__(self, nrm, kind, head):
        self.nrm, self.kind, self.head, self.m = nrm, kind, head, None

    def add(self, c):
        ss = jnp.sum(c * c, axis=1, keepdims=True)
        for g in range(0, c.shape[0], 8):
            self.m = ss[g:g + 8] if self.m is None else jnp.maximum(self.m, ss[g:g + 8])

    def flush(self):
        self.nrm[self.kind, self.head] = jnp.max(self.m)


def _kv_weights(wk, wv, slot, dst):
    a_ = jnp.concatenate([_half_words(wk[slot], 0), _half_words(wv[slot], 0)], axis=1)
    b_ = jnp.concatenate([_half_words(wk[slot], 1), _half_words(wv[slot], 1)], axis=1)
    blk = [a_[0:DC // 2], b_[0:DC // 2], a_[DC // 2:], b_[DC // 2:]]
    for i in range(7):
        _st(dst.at[i], 0, DC // 2, slice(None), _comb(blk, B_COMB[i]))


def _kv_pieces(cb, cs, bkv, kv_a, kv_b, na, nb):
    rows = CFG.get("krow", 128)

    def mk(r0):
        def prod(i):
            return jnp.dot(_left_operand(cb, cs, DC // 2, i, r0, rows), _ld(bkv.at[i], 0, DC // 2),
                           preferred_element_type=f32)

        def finish(c):
            _st(kv_a, r0, rows, slice(None), c[0])
            _st(kv_b, r0, rows, slice(None), c[1])
            _st(kv_a, S // 2 + r0, rows, slice(None), c[2])
            _st(kv_b, S // 2 + r0, rows, slice(None), c[3])
            for j in range(4):
                (na, nb)[j % 2].add(c[j][:, 0:D])

        return _strassen_steps(prod, finish, rows * 2 / 128)

    return [x for r in range(S // 2 // rows) for x in mk(r * rows)] + [(0, na.flush), (0, nb.flush)]


def _kv_plain_pieces(cb, wk, wv, slot, parity, kv_dst, rows=128):
    st = {}

    def mk(r):
        def f():
            if not st:
                st["w"] = jnp.concatenate([_head_weights(wk[slot], parity), _head_weights(wv[slot], parity)], axis=1)
            _st(kv_dst, r * rows, rows, slice(None), jnp.dot(_ld(cb, r * rows, rows), st["w"], preferred_element_type=f32))
        return f

    return [(rows * 4 / 128, mk(r)) for r in range(S // rows)]


def _q_weights(wq, slot, dst):
    e_, o_ = _half_words(wq[slot], 0), _half_words(wq[slot], 1)
    blk = [e_[0:M // 2], o_[0:M // 2], e_[M // 2:], o_[M // 2:]]
    for i in range(7):
        _st(dst.at[i], 0, M // 2, slice(None), _comb(blk, B_COMB[i]))


def _q_pieces(xa, xs, bq, q_even, q_odd, na, nb):
    rows = CFG.get("prow", 128)

    def mk(r0):
        def prod(i):
            return jnp.dot(_left_operand(xa, xs, M // 2, i, r0, rows), _ld(bq.at[i], 0, M // 2),
                           preferred_element_type=f32)

        def finish(c):
            for j in range(4):
                q = c[j] * QSCALE
                _st((q_even, q_odd)[j % 2], (S // 2) * (j // 2) + r0, rows, slice(None), q)
                (na, nb)[j % 2].add(q)

        return _strassen_steps(prod, finish, rows * 2 / 128)

    return [x for r in range(S // 2 // rows) for x in mk(r * rows)] + [(0, na.flush), (0, nb.flush)]


def _copy_rows(src, dst, r0, n):
    dst[pl.ds(r0, n), :] = src[pl.ds(r0, n), :]


def _fold(s, op):
    r = s[:, 0:128]
    for c in range(1, s.shape[1] // 128):
        r = op(r, s[:, c * 128:(c + 1) * 128])
    return r


def _recip(l):
    r = pl.reciprocal(l, approx=True)
    return r * (2.0 - l * r)


def _attention_rowmax(q_ref, kv_ref, ctx, head, sbuf):
    bq = 128

    def q_block(i, carry):
        q = _ld(q_ref, i * bq, bq)
        row = lax.broadcasted_iota(jnp.int32, (bq, bq), 0) + i * bq

        def scores(t, m):
            s = lax.dot_general(q, _ld(kv_ref, t * bq, bq, slice(0, D)), NT, preferred_element_type=f32)
            s = jnp.where(lax.broadcasted_iota(jnp.int32, (bq, bq), 1) + t * bq <= row, s, -1e9)
            sbuf[t] = s
            return jnp.maximum(m, s)

        m = lax.fori_loop(0, i + 1, scores, jnp.full((bq, bq), -jnp.inf, f32))
        m = jnp.max(m, axis=1, keepdims=True)

        def values(t, c):
            p = jnp.exp2(sbuf[t] - m)
            o = jnp.dot(p.astype(bf16), _ld(kv_ref, t * bq, bq, slice(D, 2 * D)), preferred_element_type=f32)
            return c[0] + p, c[1] + o

        lvec, acc = lax.fori_loop(0, i + 1, values, (jnp.zeros((bq, bq), f32), jnp.zeros((bq, D), f32)))
        _st(ctx.at[head], i * bq, bq, slice(None), acc / jnp.sum(lvec, axis=1, keepdims=True))
        return carry

    lax.fori_loop(0, S // bq, q_block, 0)


def _attention_bounded(q_ref, kv_ref, ctx, col0, pieces, after_round=None):
    bq = 128
    bk = CFG.get("fbk", 512)
    nq = S // bq
    fill = _Filler(pieces)
    steps = [(i, t) for i in range(nq) for t in range(((i + 1) * bq + bk - 1) // bk)]
    width = lambda i, t: min(bk, (i + 1) * bq - t * bk)
    look = CFG.get("look", 1)
    dep = CFG.get("fdep", "n")
    st = {"q": {}, "lvec": None, "acc": None, "r": {}}

    def qk(i, t):
        w = width(i, t)
        if i not in st["q"]:
            qn = _ld(q_ref, i * bq, bq)
            lag = CFG.get("lag", 2)
            if dep == "r" and (i - lag) in st["r"]:
                z = pltpu.bitcast(jnp.minimum(st["r"][i - lag], 0.0), u32)
                qn = pltpu.bitcast(pltpu.bitcast(qn, u32) | (z[0:bq // 2] | z[bq // 2:bq]), bf16)
            st["q"][i] = qn
        s = lax.dot_general(st["q"][i], _ld(kv_ref, t * bk, w, slice(0, D)), NT, preferred_element_type=f32)
        if t * bk + w - 1 > i * bq:
            row = lax.broadcasted_iota(jnp.int32, (bq, bq), 0)
            col = lax.broadcasted_iota(jnp.int32, (bq, bq), 1)
            diag = jnp.where(col <= row, s[:, w - bq:], -1e9)
            s = diag if w == bq else jnp.concatenate([s[:, :w - bq], diag], axis=1)
        return s

    def pv(i, t, s):
        w = width(i, t)
        p = jnp.exp2(s)
        f = _fold(p, jnp.add)
        st["lvec"] = f if t == 0 else st["lvec"] + f
        if dep == "pf":
            p = jnp.concatenate([jnp.maximum(p[:, 0:128], jnp.minimum(st["lvec"], 0.0))] + ([p[:, 128:]] if w > 128 else []), axis=1)
        o = jnp.dot(p.astype(bf16), _ld(kv_ref, t * bk, w, slice(D, 2 * D)), preferred_element_type=f32)
        st["acc"] = o if t == 0 else st["acc"] + o
        if (t + 1) * bk >= (i + 1) * bq:
            r = _recip(jnp.sum(st["lvec"], axis=1, keepdims=True))
            _st(ctx.at[col0], i * bq, bq, slice(None), st["acc"] * r)
            st["r"][i] = jnp.broadcast_to(r, (bq, 128))
            if after_round is not None:
                after_round(i, fill)

    fill.upto(CFG.get("lead0", 0.0))
    pend = []
    for n, (i, t) in enumerate(steps):
        pend.append((i, t, qk(i, t)))
        fill.upto(((n + 1) / len(steps)) ** CFG.get("alpha", 1.0))
        if len(pend) > look:
            pv(*pend.pop(0))
    for x in pend:
        pv(*x)
    fill.upto(1.0)


OROW = 512


def _kernel(x_h, c_h, wq_h, wk_h, wv_h, wo_h, xb_h, wr_h, wi_h, dfw_h, div_h, tm_h, tmi_h, ids, out_h,
            xa, cb, xs, cs, wq, wk, wv, wo, wos, qa, kva, qb, kvb, qt, kte, kto, bq, bkv, ctx, pbuf, sbuf, nrm,
            xb, wtr, wti, wnr, wni, dfw, div, tm, tmi, wbr, wbi,
            sem_a, sem_w, sem_b, sem_c, sem_o):
    phases = CFG.get("phases", "plLod")
    pr, pi = _PView(pbuf, 0), _PView(pbuf, 10)
    w32 = lambda ref: ref.bitcast(u32)

    def tile_ids(t):
        if not CFG.get("opq", 1):
            return [t] * 6
        return [ids[s, t] for s in range(6)]

    def wcopies(pair, slot):
        return (pltpu.make_async_copy(w32(wk_h).at[:, pair, :], wk.at[slot], sem_w.at[slot, 0]),
                pltpu.make_async_copy(w32(wv_h).at[:, pair, :], wv.at[slot], sem_w.at[slot, 1]),
                pltpu.make_async_copy(w32(wq_h).at[:, pair, :], wq.at[slot], sem_w.at[slot, 2]))

    c_cps = [pltpu.make_async_copy(w32(c_h).at[r * 256:(r + 1) * 256, :], cb.at[r * 256:(r + 1) * 256, :], sem_a.at[r])
             for r in range(4)]
    x_cps = [pltpu.make_async_copy(w32(x_h).at[r * 256:(r + 1) * 256, :], xa.at[r * 256:(r + 1) * 256, :], sem_a.at[4 + r])
             for r in range(4)]
    b_cps = [pltpu.make_async_copy(a, b, sem_b.at[i]) for i, (a, b) in enumerate(
        ((w32(dfw_h), dfw), (wr_h.at[512:513, :], wnr), (wi_h.at[512:513, :], wni),
         (w32(div_h), div), (w32(tm_h), tm), (w32(tmi_h), tmi)))]

    def bcopies(j):
        rows = pl.ds(_mo(j * 64, 64), 64)
        lanes = pl.ds(_mo(j * 128, 128), 128)
        return (pltpu.make_async_copy(w32(xb_h).at[rows, :], xb.at[rows, :], sem_c.at[j, 0]),
                pltpu.make_async_copy(wr_h.at[0:512, lanes], wtr.at[j], sem_c.at[j, 1]),
                pltpu.make_async_copy(wi_h.at[0:512, lanes], wti.at[j], sem_c.at[j, 2]))

    def wocopies(j):
        out = []
        for hf in range(2):
            rows = pl.ds(_mo(hf * (H * D // 4) + j * 64, 64), 64)
            out.append(pltpu.make_async_copy(w32(wo_h).at[rows, :], wo.at[rows, :], sem_c.at[j, 3 + hf]))
        return tuple(out)

    def wo_sums(j):
        blk = [_ld(wo, (b // 2) * (H * D // 2) + j * 128, 128, slice((b % 2) * (M // 2), (b % 2 + 1) * (M // 2))).astype(f32)
               for b in range(4)]
        for s_, i in enumerate(B_SUMS):
            _st(wos.at[s_], j * 128, 128, slice(None), _comb(blk, B_COMB[i]))

    w0 = wcopies(0, 0)
    first_norms = [_RowNorm(nrm, kind, h) for kind in range(2) for h in range(2)]

    def kv_first(r):
        if "p" not in phases:
            return
        w = jnp.concatenate([_head_weights(x_[0], par) for par in range(2) for x_ in (wk, wv)], axis=1)
        for j in (2 * r, 2 * r + 1):
            kv = jnp.dot(_ld(cb, j * 256, 256), w, preferred_element_type=f32)
            _st(kva, j * 256, 256, slice(None), kv[:, 0:2 * D])
            _st(kto, j * 256, 256, slice(None), kv[:, 2 * D:4 * D])
            first_norms[2].add(kv[:, 0:D]); first_norms[3].add(kv[:, 2 * D:3 * D])

    def q_first(r):
        if "p" not in phases:
            return
        w = jnp.concatenate([_head_weights(wq[0], 0), _head_weights(wq[0], 1)], axis=1)
        for j in (2 * r, 2 * r + 1):
            q = jnp.dot(_ld(xa, j * 256, 256), w, preferred_element_type=f32) * QSCALE
            _st(qa, j * 256, 256, slice(None), q[:, 0:D])
            _st(qt, j * 256, 256, slice(None), q[:, D:2 * D])
            first_norms[0].add(q[:, 0:D]); first_norms[1].add(q[:, D:2 * D])

    order = (0, 2, 1, 3)
    w0[0].start(); w0[1].start(); c_cps[0].start(); c_cps[2].start(); c_cps[1].start()
    with _scope("wait_c"):
        w0[0].wait(); w0[1].wait(); c_cps[0].wait()
    c_cps[3].start(); w0[2].start(); x_cps[0].start()
    for cp in b_cps[:3]:
        cp.start()
    with _scope("kvproj0"):
        for n, r in enumerate(order):
            if n > 0:
                c_cps[r].wait(); x_cps[r].start()
            if n % 2 == 1 and "p" in phases:
                _left_sums(cb, cs, DC // 2, (n // 2) * 512, 512)
            kv_first(r)
    with _scope("qproj0"):
        w0[2].wait()
        for n, r in enumerate(order):
            x_cps[r].wait()
            if n == CFG.get("w1r", 2):
                for cp in wcopies(1, 1):
                    cp.start()
            if n % 2 == 1 and "p" in phases:
                _left_sums(xa, xs, M // 2, (n // 2) * 512, 512)
            q_first(r)
    for cp in list(wcopies(2, 2)) + b_cps[3:] + list(bcopies(0)) + list(wocopies(0)):
        cp.start()
    for cp in wcopies(1, 1):
        cp.wait()
    if "p" in phases:
        _kv_weights(wk, wv, 1, bkv)
        for n_ in first_norms:
            n_.flush()
    else:
        for k_ in range(2):
            for h_ in range(H):
                nrm[k_, h_] = 0.0

    def step_copies(p, last):
        if not last:
            for cp in wcopies(lax.min(p + 2, H // 2 - 1), (p + 2) & 3):
                cp.wait()
        for cp in bcopies(p) + wocopies(p):
            cp.wait()
        if not last:
            for cp in wcopies(lax.min(p + 3, H // 2 - 1), (p + 3) & 3) + bcopies(p + 1) + wocopies(p + 1):
                cp.start()

    def side_pieces(p):
        bp = [(3.5, functools.partial(_d_fwd, xb, dfw, pr, pi, p * 128, 128)), (1, functools.partial(wo_sums, p))]
        return bp + [(0.5, functools.partial(_w_prep, wt, wn, wb, t, p))
                     for t in range(5) for (wt, wn, wb) in ((wtr, wnr, wbr), (wti, wni, wbi))]

    def spread(base, extra):
        step = max(1, len(base) // (len(extra) + 1))
        out_, extra = [], list(extra)
        for n, piece in enumerate(base):
            if n % step == step - 1 and extra:
                out_.append(extra.pop(0))
            out_.append(piece)
        return out_ + extra

    def copies(src, dst, cost):
        return [(cost, functools.partial(_copy_rows, src, dst, r * 256, 256)) for r in range(4)]

    def bounded(p):
        lim = SAFE_LOG2 ** 2 / 1.05
        return jnp.logical_and(nrm[0, 2 * p] * nrm[1, 2 * p] <= lim, nrm[0, 2 * p + 1] * nrm[1, 2 * p + 1] <= lim)

    def pair_fast(p, last):
        step_copies(p, last)
        fa = copies(qt, qb, 0.5) + copies(kto, kvb, 1)
        if last:
            fa += side_pieces(p) + _s_fwd(pr, pi, tile_ids(0))
        else:
            fa += _kv_pieces(cb, cs, bkv, kte, kto, _RowNorm(nrm, 1, 2 * p + 2), _RowNorm(nrm, 1, 2 * p + 3))
            fa += [(1, functools.partial(_q_weights, wq, (p + 1) & 3, bq))]
            fa = spread(fa, side_pieces(p))
        _attention_bounded(qa, kva, ctx, 2 * p, fa)
        hook = None
        if last:
            fb = [(1, lambda: None)]

            def hook(i, fill):
                if i == OROW // 128 - 1:
                    fill.insert([(1, functools.partial(ctx_sum, 0, s_, c0, c0 + 4)) for s_ in range(5) for c0 in range(0, H // 2, 4)])
        else:
            fb = copies(kte, kva, 1) + _q_pieces(xa, xs, bq, qa, qt, _RowNorm(nrm, 0, 2 * p + 2), _RowNorm(nrm, 0, 2 * p + 3))
            fb += [(1, functools.partial(_kv_weights, wk, wv, (p + 2) & 3, bkv))]
        _attention_bounded(qb, kvb, ctx, 2 * p + 1, fb, hook)

    def pair_general(p, last):
        step_copies(p, last)
        for _, f in copies(qt, qb, 0) + copies(kto, kvb, 0) + side_pieces(p):
            f()
        _attention_rowmax(qa, kva, ctx, 2 * p, sbuf)
        _attention_rowmax(qb, kvb, ctx, 2 * p + 1, sbuf)
        if last:
            for _, f in _s_fwd(pr, pi, tile_ids(0)):
                f()
            for s_ in range(5):
                ctx_sum(0, s_)
            return
        slot = (p + 1) & 3

        def proj(j, carry):
            wkv = jnp.concatenate([_head_weights(x_[slot], par) for par in range(2) for x_ in (wk, wv)], axis=1)
            kv = jnp.dot(_ld(cb, j * 256, 256), wkv, preferred_element_type=f32)
            _st(kva, j * 256, 256, slice(None), kv[:, 0:2 * D])
            _st(kto, j * 256, 256, slice(None), kv[:, 2 * D:4 * D])
            w = jnp.concatenate([_head_weights(wq[slot], 0), _head_weights(wq[slot], 1)], axis=1)
            q = jnp.dot(_ld(xa, j * 256, 256), w, preferred_element_type=f32) * QSCALE
            _st(qa, j * 256, 256, slice(None), q[:, 0:D])
            _st(qt, j * 256, 256, slice(None), q[:, D:2 * D])
            return carry

        lax.fori_loop(0, S // 256, proj, 0)

    def ctx_row0(r, half):
        return _mo(r * OROW + half * (OROW // 2), OROW // 2)

    def ctx_block(r, b, c0, nc):
        return jnp.concatenate([_ld(ctx.at[(b % 2) * (H // 2) + c], ctx_row0(r, b // 2), OROW // 2)
                                for c in range(c0, c0 + nc)], axis=1)

    def ctx_sum(r, s_, lo=0, hi=H // 2):
        terms = A_COMB[A_SUMS[s_]]
        g = CFG.get("cgran", 64)
        for c in range(lo, hi):
            for r0 in range(0, OROW // 2, g):
                blk = {b: _ld(ctx.at[(b % 2) * (H // 2) + c], ctx_row0(r, b // 2) + r0, g).astype(f32) for b, _ in terms}
                _st(xs.at[s_], (c // 4) * 256 + r0, g, slice((c % 4) * D, (c % 4 + 1) * D), _comb(blk, terms))

    LAST = H // 2 - 1
    for cp in b_cps[:3]:
        cp.wait()
    with _scope("mainloop"):
        if "l" in phases:
            def fast_step(p):
                pair_fast(p, False)
                return p + 1

            def more(p):
                return jnp.logical_and(p < LAST, bounded(lax.min(p, LAST)))

            p_stop = lax.while_loop(more, fast_step, jnp.int32(0))
        else:
            p_stop = jnp.int32(0)

    def general_step(p, carry):
        pair_general(p, False)
        return carry

    lax.fori_loop(p_stop, LAST, general_step, 0)
    for cp in wcopies(LAST, 1):
        cp.wait()
    for cp in b_cps[3:]:
        cp.wait()
    with _scope("peeled"):
        if "L" in phases:
            ok = jnp.logical_and(p_stop == LAST, bounded(LAST))

            @pl.when(ok)
            def _():
                pair_fast(LAST, True)

            @pl.when(jnp.logical_not(ok))
            def _():
                pair_general(LAST, True)
        else:
            step_copies(LAST, True)

    def out_copy(r):
        rows = pl.ds(r * (OROW // 2), OROW // 2)
        return pltpu.make_async_copy(xa.at[rows, :], w32(out_h).at[rows, 0:M], sem_o.at[r])

    def out_body(r, carry):
        rest = _s_rest(pr, pi, tm, tmi, wbr, wbi, tile_ids(r))
        fwd = _s_fwd(pr, pi, tile_ids(r + 1))
        fo = CFG.get("fwdorder", 0)
        pieces = (rest + fwd) if fo == 0 else (fwd + rest) if fo == 1 else (rest[:R] + fwd + rest[R:])
        fill = _Filler(pieces)
        ksub = 512
        nk = (H * D // 2) // ksub
        cnt = [0]
        nxt = lax.min(r + 1, S // OROW - 1)

        def prod(i):
            acc = None
            for jk in range(nk):
                if i in A_SUMS:
                    lhs = _ld(xs.at[A_SUMS.index(i)], jk * 256, 256)
                else:
                    lhs = ctx_block(r, A_COMB[i][0][0], jk * ksub // D, ksub // D)
                if i in B_SUMS:
                    rhs = _ld(wos.at[B_SUMS.index(i)], jk * ksub, ksub)
                else:
                    b = B_COMB[i][0][0]
                    rhs = _ld(wo, (b // 2) * (H * D // 2) + jk * ksub, ksub, slice((b % 2) * (M // 2), (b % 2 + 1) * (M // 2)))
                o = jnp.dot(lhs, rhs, preferred_element_type=f32)
                acc = o if acc is None else acc + o
                cnt[0] += 1
                fill.upto(cnt[0] / (7 * nk))
            if i in A_SUMS:
                ctx_sum(nxt, A_SUMS.index(i))
            return acc

        def finish(c):
            for j in range(4):
                _st(xa, ctx_row0(r, j // 2), OROW // 2, slice((j % 2) * (M // 2), (j % 2 + 1) * (M // 2)), c[j])

        for _, f in _strassen_steps(prod, finish, 0):
            f()
        fill.upto(1.0)
        out_copy(r).start()
        return carry

    with _scope("outloop"):
        if "o" in phases:
            lax.fori_loop(0, S // OROW, out_body, 0)
        else:
            for r in range(S // OROW):
                out_copy(r).start()

    if "d" in phases:
        for _, f in _s_rest(pr, pi, tm, tmi, wbr, wbi, tile_ids(4)):
            f()
    if phases != "plLod":
        for n, ref in enumerate((pbuf, wos, ctx, bq, bkv, xs, cs)):
            cp = pltpu.make_async_copy(ref.at[0, 0:8, 0:128], w32(out_h).at[0:8, 0:128], sem_o.at[8 + n])
            cp.start(); cp.wait()
        for n, ref in enumerate((wbr, wbi)):
            cp = pltpu.make_async_copy(ref.at[0, 0:16, :], out_h.at[0:16, 0:128], sem_o.at[16 + n])
            cp.start(); cp.wait()
    nchunk = CFG.get("ychunk", 8)
    ycp = []
    with _scope("dinv"):
        for r in range(nchunk):
            for j in range(S // nchunk // 128):
                if "d" in phases:
                    _d_inv(pr, pi, div, xb, r * (S // nchunk) + j * 128, 128)
            rows = slice(r * (S // nchunk // 2), (r + 1) * (S // nchunk // 2))
            cp = pltpu.make_async_copy(xb.at[rows, :], w32(out_h).at[rows, M:M + DD], sem_o.at[4 + r])
            cp.start()
            ycp.append(cp)
    with _scope("finalwait"):
        for r in range(S // OROW):
            out_copy(r).wait()
        for cp in ycp:
            cp.wait()


def _flags():
    fl = {}
    if CFG.get("lp"):
        fl["XLA_TPU_FORCE_LP_LLO_SCHEDULER"] = True
    if CFG.get("even"):
        fl["XLA_TPU_EVENLY_DISTRIBUTE_CRITICAL_NODES"] = True
    return fl or None


@jax.jit
def pallas_concat_heads__compressed_kv_cla__spectral_gfnet__prompt_kernel(
        A_x, A_c_kv, A_w_q, A_w_uk, A_w_uv, A_w_o, B_x, B_w_r, B_w_i):
    dfw, div, tm, tmi = _dft_consts()
    hbm = pl.BlockSpec(memory_space=pl.ANY)
    vm = pltpu.VMEM
    scratch = [
        vm((S // 2, M), u32), vm((S // 2, DC), u32), vm((5, S // 4, M // 2), u32), vm((5, S // 4, DC // 2), u32),
        vm((4, M, D), u32), vm((4, DC, D), u32), vm((4, DC, D), u32), vm((H * D // 2, M), u32), vm((5, H * D // 4, M // 2), u32),
        vm((S // 2, D), u32), vm((S // 2, 2 * D), u32), vm((S // 2, D), u32), vm((S // 2, 2 * D), u32), vm((S // 2, D), u32), vm((S // 2, 2 * D), u32), vm((S // 2, 2 * D), u32),
        vm((7, M // 4, D), u32), vm((7, DC // 4, 2 * D), u32),
        vm((H, S // 2, D), u32), vm((20, S // 2, D), u32), vm((16, 128, 128), f32), pltpu.SMEM((2, H), f32),
        vm((S // 2, DD), u32), vm((16, 512, 128), bf16), vm((16, 512, 128), bf16), vm((1, S), bf16), vm((1, S), bf16),
        vm((512, 256), u32), vm((512, 256), u32), vm((R * 64, 128), u32), vm((R * 64, 128), u32),
        vm((5, S, 128), bf16), vm((5, S, 128), bf16),
        pltpu.SemaphoreType.DMA((9,)), pltpu.SemaphoreType.DMA((4, 3)),
        pltpu.SemaphoreType.DMA((9,)), pltpu.SemaphoreType.DMA((16, 5)), pltpu.SemaphoreType.DMA((4 + 16,)),
    ]
    out = pl.pallas_call(
        _kernel,
        out_shape=jax.ShapeDtypeStruct((S, M + DD), bf16),
        in_specs=[hbm] * 13 + [pl.BlockSpec(memory_space=pltpu.SMEM)],
        out_specs=hbm,
        scratch_shapes=scratch,
        compiler_params=pltpu.CompilerParams(vmem_limit_bytes=124 * 1024 * 1024, flags=_flags(),
                                             shape_invariant_numerics=not CFG.get('sin', 0)),
        name="mla_gfnet",
    )(A_x.reshape(S, M), A_c_kv.reshape(S, DC), A_w_q, A_w_uk, A_w_uv, A_w_o.reshape(H * D, M),
      B_x.reshape(S, DD), B_w_r.T, B_w_i.T,
      jnp.asarray(dfw), jnp.asarray(div), jnp.asarray(tm), jnp.asarray(tmi),
      jnp.asarray(np.tile(np.arange(8, dtype=np.int32), (6, 1))))
    return out.reshape(1, S, M + DD)
```
